```python
import os as _os
_os.environ.setdefault("JAX_PLATFORMS", "cpu")
import jax
import jax.numpy as jnp

def _softmax(x, axis=-1):
    return jax.nn.softmax(x, axis=axis)
def _gelu(x):
    return jax.nn.gelu(x, approximate=True)
def _silu(x):
    return jax.nn.silu(x)
def _sigmoid(x):
    return jax.nn.sigmoid(x)
def _layernorm(x, axis=-1, eps=1e-5):
    m = jnp.mean(x, axis=axis, keepdims=True)
    v = jnp.var(x, axis=axis, keepdims=True)
    return (x - m) / jnp.sqrt(v + eps)
def _scatter_add(tgt, idx, src, axis=0):
    return tgt.at[idx].add(src)
def _segment_sum(src, seg, n):
    return jax.ops.segment_sum(src, seg, n)
class _Rng:
    def __init__(self, key):
        self._k = key
    def _next(self):
        self._k, sub = jax.random.split(self._k)
        return sub
    def normal(self, shape):
        return jax.random.normal(self._next(), shape, dtype=jnp.bfloat16)
    def randint(self, lo, hi, shape):
        return jax.random.randint(self._next(), shape, lo, hi, dtype=jnp.int32)
    def uniform(self, shape, lo=0.0, hi=1.0):
        return jax.random.uniform(self._next(), shape, jnp.bfloat16, lo, hi)
    def permutation(self, n):
        return jax.random.permutation(self._next(), n)


kernel_name = 'concat_heads__gqa_block_cached__gqa_block_cached__near_ridge'

def setup_inputs():
    _rng = _Rng(jax.random.key(int.from_bytes(__import__("os").urandom(4), "little")))
    _w = (lambda a: (lambda t: t.astype(jnp.bfloat16) if jnp.issubdtype(t.dtype, jnp.floating) else t)(jnp.asarray(a)))
    def _A_setup():
        B, Sq, D = 32, 48, 512
        Hq, Hkv, Sk, Dh = 32, 32, 48, 128
        assert Hq % Hkv == 0, (Hq, Hkv)
        return {
            "x": _w((lambda *s: _rng.normal(s) * 0.8)(B, Sq, D)),
            "k_cache": _w((lambda *s: _rng.normal(s) * 0.8)(B, Hkv, Sk, Dh)),
            "v_cache": _w((lambda *s: _rng.normal(s) * 0.05)(B, Hkv, Sk, Dh)),
            "wq": _w((lambda *s: _rng.normal(s) * 0.8)(D, Hq * Dh) * (D ** -0.5)),
            "wo": _w((lambda *s: _rng.normal(s) * 0.05)(Hq * Dh, D) * ((Hq * Dh) ** -0.5)),
        }
    _A_in = _A_setup()

    def _B_setup():
        B, Sq, D = 32, 48, 512
        Hq, Hkv, Sk, Dh = 32, 32, 48, 128
        assert Hq % Hkv == 0, (Hq, Hkv)
        return {
            "x": _w((lambda *s: _rng.normal(s) * 0.8)(B, Sq, D)),
            "k_cache": _w((lambda *s: _rng.normal(s) * 0.8)(B, Hkv, Sk, Dh)),
            "v_cache": _w((lambda *s: _rng.normal(s) * 0.05)(B, Hkv, Sk, Dh)),
            "wq": _w((lambda *s: _rng.normal(s) * 0.8)(D, Hq * Dh) * (D ** -0.5)),
            "wo": _w((lambda *s: _rng.normal(s) * 0.05)(Hq * Dh, D) * ((Hq * Dh) ** -0.5)),
        }
    _B_in = _B_setup()

    return {
        "A_x": _A_in["x"],
        "A_k_cache": _A_in["k_cache"],
        "A_v_cache": _A_in["v_cache"],
        "A_wq": _A_in["wq"],
        "A_wo": _A_in["wo"],
        "B_x": _B_in["x"],
        "B_k_cache": _B_in["k_cache"],
        "B_v_cache": _B_in["v_cache"],
        "B_wq": _B_in["wq"],
        "B_wo": _B_in["wo"],
    }

def reference(A_x, A_k_cache, A_v_cache, A_wq, A_wo, B_x, B_k_cache, B_v_cache, B_wq, B_wo):
    def _A_ref(x, k_cache, v_cache, wq, wo):
        B, Sq, D = x.shape
        Hq, Dh = 32, 128
        Hkv = k_cache.shape[1]
        rep = Hq // Hkv
        q = (lambda x, *d: x.transpose(*d))((x @ wq).reshape(B, Sq, Hq, Dh), 0, 2, 1, 3)
        k = jnp.repeat(k_cache, rep, axis=1)
        v = jnp.repeat(v_cache, rep, axis=1)
        scores = jnp.einsum("bhqd,bhkd->bhqk", q, k) * (Dh ** -0.5)
        p = _softmax(scores, axis=-1)
        o = jnp.einsum("bhqk,bhkd->bhqd", p, v)
        return (lambda x, *d: x.transpose(*d))(o, 0, 2, 1, 3).reshape(B, Sq, Hq * Dh) @ wo

    def _B_ref(x, k_cache, v_cache, wq, wo):
        B, Sq, D = x.shape
        Hq, Dh = 32, 128
        Hkv = k_cache.shape[1]
        rep = Hq // Hkv
        q = (lambda x, *d: x.transpose(*d))((x @ wq).reshape(B, Sq, Hq, Dh), 0, 2, 1, 3)
        k = jnp.repeat(k_cache, rep, axis=1)
        v = jnp.repeat(v_cache, rep, axis=1)
        scores = jnp.einsum("bhqd,bhkd->bhqk", q, k) * (Dh ** -0.5)
        p = _softmax(scores, axis=-1)
        o = jnp.einsum("bhqk,bhkd->bhqd", p, v)
        return (lambda x, *d: x.transpose(*d))(o, 0, 2, 1, 3).reshape(B, Sq, Hq * Dh) @ wo

    a = _A_ref(A_x, A_k_cache, A_v_cache, A_wq, A_wo)
    b = _B_ref(B_x, B_k_cache, B_v_cache, B_wq, B_wo)
    return jnp.concatenate([a, b], axis=-1)
```

```python
import functools, os
import jax
import jax.numpy as jnp
from jax import lax
import jax.experimental.pallas as pl
import jax.experimental.pallas.tpu as pltpu

B = 32
H = 32
SQ = 48
DH = 128
D = 512
HG = int(os.environ.get("HG", 4))
G = int(os.environ.get("G", 4))
OPLAG = int(os.environ.get("OPLAG", 2))
NG = B // G
NIT = H // HG
M = G * SQ
ROWS = B * SQ
QSCALE = (DH ** -0.5) * 1.4426950408889634
bf16 = jnp.bfloat16
f32 = jnp.float32


def _softmax_p(s):
    m = jnp.max(s, axis=-1, keepdims=True)
    e = jnp.exp2(s - m)
    l = jnp.sum(e, axis=-1, keepdims=True)
    return (e * pl.reciprocal(l, approx=True)).astype(bf16)


def _iter_body(x_v, wq_v, wo_v, k_v, v_v, q_s, o_s, acc, out_v):
    def qp(g, n):
        rows = pl.ds(g * M, M)
        q = jnp.dot(x_v[rows, :], wq_v[:, n * DH:(n + 1) * DH], preferred_element_type=f32)
        q_s[rows, n * DH:(n + 1) * DH] = (q * QSCALE).astype(bf16)

    def qk(g, n):
        ps = []
        for j in range(G):
            b = g * G + j
            qh = q_s[b * SQ:(b + 1) * SQ, n * DH:(n + 1) * DH]
            s = lax.dot_general(qh, k_v[b, n], (((1,), (1,)), ((), ())), preferred_element_type=f32)
            ps.append(s)
        return [_softmax_p(s) for s in ps]

    def pv(g, n, ps):
        for j in range(G):
            b = g * G + j
            o = jnp.dot(ps[j], v_v[b, n], preferred_element_type=f32)
            o_s[b * SQ:(b + 1) * SQ, n * DH:(n + 1) * DH] = o.astype(bf16)

    NT = D // 128
    def op(g, t):
        rows = pl.ds(g * M, M)
        cols = slice(t * 128, (t + 1) * 128)
        r = acc[rows, cols] + jnp.dot(o_s[rows, :], wo_v[:, cols], preferred_element_type=f32)
        acc[rows, cols] = r
        out_v[rows, cols] = r.astype(bf16)

    pend = None
    for s in range(NG + 1 + OPLAG):
        for n in range(HG):
            if s < NG:
                qp(s, n)
            new = None
            if 1 <= s <= NG:
                new = (s - 1, n, qk(s - 1, n))
            go = s - 1 - OPLAG
            if 0 <= go < NG:
                for t in range(n * NT // HG, (n + 1) * NT // HG):
                    op(go, t)
            if pend is not None:
                pv(*pend)
            pend = new
    assert pend is None


def _body(ax, ak, av, awq, awo, bx, bk, bv, bwq, bwo, out_hbm,
          x_v, wq_v, wo_v, k_v, v_v, q_s, o_s, acc, out_v, sem_x, sem_in, sem_out):
    srcs = ((ax, ak, av, awq, awo), (bx, bk, bv, bwq, bwo))

    def in_copies(br, hg, slot):
        _, k, v, wq, wo = srcs[br]
        return [
            pltpu.make_async_copy(wq.at[:, pl.ds(hg * HG * DH, HG * DH)], wq_v.at[slot], sem_in.at[slot, 0]),
            pltpu.make_async_copy(k.at[:, pl.ds(hg * HG, HG)], k_v.at[slot], sem_in.at[slot, 1]),
            pltpu.make_async_copy(v.at[:, pl.ds(hg * HG, HG)], v_v.at[slot], sem_in.at[slot, 2]),
            pltpu.make_async_copy(wo.at[pl.ds(hg * HG * DH, HG * DH), :], wo_v.at[slot], sem_in.at[slot, 3]),
        ]

    def x_copy(br):
        return pltpu.make_async_copy(srcs[br][0], x_v.at[br], sem_x.at[br])

    def out_copy(br):
        return pltpu.make_async_copy(out_v.at[br], out_hbm.at[:, pl.ds(br * D, D)], sem_out.at[br])

    x_copy(0).start()
    for c in in_copies(0, 0, 0):
        c.start()
    x_copy(1).start()
    acc[...] = jnp.zeros(acc.shape, f32)
    x_copy(0).wait()
    x_copy(1).wait()

    def step(it, carry):
        slot = it % 2
        br = it // NIT
        nxt = it + 1

        @pl.when(nxt < NIT)
        def _():
            for c in in_copies(0, nxt, 1 - slot):
                c.start()

        @pl.when(jnp.logical_and(nxt >= NIT, nxt < 2 * NIT))
        def _():
            for c in in_copies(1, nxt - NIT, 1 - slot):
                c.start()

        for c in in_copies(0, 0, slot):
            c.wait()

        _iter_body(x_v.at[br], wq_v.at[slot], wo_v.at[slot], k_v.at[slot], v_v.at[slot],
                   q_s, o_s, acc.at[br], out_v.at[br])

        @pl.when(it == NIT - 1)
        def _():
            out_copy(0).start()
        return carry

    lax.fori_loop(0, 2 * NIT, step, 0)
    out_copy(1).start()
    out_copy(0).wait()
    out_copy(1).wait()


@jax.jit
def pallas_concat_heads__gqa_block_cached__gqa_block_cached__near_ridge_kernel(A_x, A_k_cache, A_v_cache, A_wq, A_wo, B_x, B_k_cache, B_v_cache, B_wq, B_wo):
    A_k, A_v, B_k, B_v = A_k_cache, A_v_cache, B_k_cache, B_v_cache
    any_spec = pl.BlockSpec(memory_space=pl.ANY)
    out = pl.pallas_call(
        _body,
        in_specs=[any_spec] * 10,
        out_specs=any_spec,
        out_shape=jax.ShapeDtypeStruct((ROWS, 2 * D), bf16),
        scratch_shapes=[
            pltpu.VMEM((2, ROWS, D), bf16),
            pltpu.VMEM((2, D, HG * DH), bf16),
            pltpu.VMEM((2, HG * DH, D), bf16),
            pltpu.VMEM((2, B, HG, SQ, DH), bf16),
            pltpu.VMEM((2, B, HG, SQ, DH), bf16),
            pltpu.VMEM((ROWS, HG * DH), bf16),
            pltpu.VMEM((ROWS, HG * DH), bf16),
            pltpu.VMEM((2, ROWS, D), f32),
            pltpu.VMEM((2, ROWS, D), bf16),
            pltpu.SemaphoreType.DMA((2,)),
            pltpu.SemaphoreType.DMA((2, 4)),
            pltpu.SemaphoreType.DMA((2,)),
        ],
        compiler_params=pltpu.CompilerParams(vmem_limit_bytes=100 * 1024 * 1024),
    )(A_x.reshape(ROWS, D), A_k, A_v, A_wq, A_wo, B_x.reshape(ROWS, D), B_k, B_v, B_wq, B_wo)
    return out.reshape(B, SQ, 2 * D)
```

```python
import jax
import jax.numpy as jnp
from jax import lax
import jax.experimental.pallas as pl
import jax.experimental.pallas.tpu as pltpu

B = 32
H = 32
SQ = 48
DH = 128
D = 512
HC = 4
G = 4
NCI = 2
PC = 4
LL = 1
LP = 3
LO = 2
TAILR = 4

NG = B // G
NCB = H // HC
NCH = 2 * NCB
NIT = NCH // NCI
ITB = NCB // NCI
M = G * SQ
HM = M // 2
ROWS = B * SQ
CW = HC * DH
NU = NG * HC
QG = (NCH - PC) * NG // NIT
QRING = 64
NWQ = (NCH - PC) // NCI
XB_IT = 2
SCALE_LOG2E = (DH ** -0.5) * 1.4426950408889634
WAVES = ((2, 1), (3, 2), (4, 3), (5, 5), (8, 8), (2 * NG, PC * HC))

assert QG * NIT == (NCH - PC) * NG and ITB == 4 and NG == 8 and NCB * NG == 64
assert PC * NG + QG <= QRING
for _it in range(NIT):
    _last = PC * NG + QG * (_it + 1) - 1
    assert _last // NG < PC + NCI * (_it + 1)
    assert _it >= XB_IT or _last < NCB * NG

bf16 = jnp.bfloat16
f32 = jnp.float32


def _softmax(s):
    m = jnp.max(s, axis=-1, keepdims=True)
    e = jnp.exp2((s - m) * SCALE_LOG2E)
    l = jnp.sum(e, axis=-1, keepdims=True)
    r = pl.reciprocal(l, approx=True)
    r = r * (2.0 - l * r)
    return (e * r).astype(bf16)


def _loop_order():
    def units(kind):
        return [(kind, c, u // HC, u % HC) for c in range(NCI) for u in range(NU)]
    streams = ((0, units('S')), (-LL, units('L')),
               (0, [('Q', 0, j // HC, j % HC) for j in range(QG * HC)]),
               (LP + HC - 1 + LO, units('O')), (LP, units('P')))
    order = []
    for k in range(-LL, max(off + len(items) for off, items in streams)):
        for off, items in streams:
            if 0 <= k - off < len(items):
                order.append(items[k - off])
    return order


def _body(ax, ak, av, awq, awo, bx, bk, bv, bwq, bwo, out_hbm,
          x_v, wq_v, wo_v, k_v, v_v, q_s, o_s, acc, out_v, sem_in, sem_out):
    srcs = ((ax, ak, av, awq, awo), (bx, bk, bv, bwq, bwo))
    copy = pltpu.make_async_copy

    def wave_copies(i):
        r0, h0 = WAVES[i - 1] if i else (0, 0)
        r1, h1 = WAVES[i]
        sem = sem_in.at[NIT + 1 + i]
        cps = []
        while h0 < h1:
            e = min(h1, (h0 // HC + 1) * HC)
            cps.append(copy(awq.at[:, pl.ds(h0 * DH, (e - h0) * DH)],
                            wq_v.at[h0 // HC, :, pl.ds((h0 % HC) * DH, (e - h0) * DH)], sem))
            h0 = e
        rows = pl.ds(r0 * HM, (r1 - r0) * HM)
        return cps + [copy(ax.at[rows], x_v.at[0, rows], sem)]

    def xb_copy():
        return copy(bx, x_v.at[1], sem_in.at[NIT])

    def out_copy(br, row0, nrows, col0, ncols):
        rows = pl.ds(row0, nrows)
        return copy(out_v.at[br, rows, pl.ds(col0, ncols)],
                    out_hbm.at[rows, pl.ds(pl.multiple_of(br * D + col0, DH), ncols)], sem_out.at[br])

    def out_pieces(g, n):
        if g < NG - 1:
            return [(g * M, M, 0, D)] if n == HC - 1 else []
        if n < HC - 1:
            return [(g * M, M, n * DH, DH)]
        return [(g * M + i * (M // TAILR), M // TAILR, n * DH, DH) for i in range(TAILR)]

    def q_item(br, c, row0, n, slot, r0=0, nr=M):
        cols = slice(n * DH, (n + 1) * DH)
        q = jnp.dot(x_v[br, pl.ds(row0, nr), :], wq_v[c, :, cols], preferred_element_type=f32)
        q_s[slot, r0:r0 + nr, cols] = q.astype(bf16)

    for i in range(len(WAVES)):
        for cp in wave_copies(i):
            cp.start()
    for it in range(NIT):
        sem = sem_in.at[it]
        if it == XB_IT:
            xb_copy().start()
        if it < NWQ:
            for c in range(PC + it * NCI, PC + (it + 1) * NCI):
                copy(srcs[c // NCB][3].at[:, pl.ds((c % NCB) * CW, CW)], wq_v.at[c], sem).start()
        br, hc = it // ITB, (it % ITB) * NCI
        heads = pl.ds(hc * HC, NCI * HC)
        copy(srcs[br][1].at[:, heads], k_v.at[it], sem).start()
        copy(srcs[br][2].at[:, heads], v_v.at[it], sem).start()
        copy(srcs[br][4].at[pl.ds(hc * CW, NCI * CW), :], wo_v.at[it], sem).start()

    done = set()
    for i, (nr, nh) in enumerate(WAVES):
        for cp in wave_copies(i):
            cp.wait()
        for c, g, n in sorted((h // HC, g, h % HC) for h in range(nh) for g in range((nr + 1) // 2)):
            halves = [a for a in range(2) if 2 * g + a < nr and (c, g, n, a) not in done]
            if halves:
                q_item(0, c, g * M + halves[0] * HM, n, c * NG + g, halves[0] * HM, len(halves) * HM)
                done.update((c, g, n, a) for a in halves)

    order = _loop_order()

    def step(it, carry):
        sem = sem_in.at[it]
        need_wq, need_xb = it < NWQ, it == XB_IT
        for dst in (k_v.at[it], v_v.at[it], wo_v.at[it]):
            copy(dst, dst, sem).wait()

        @pl.when(need_wq)
        def _():
            dst = wq_v.at[pl.ds(jnp.minimum(PC + it * NCI, NCH - NCI), NCI)]
            copy(dst, dst, sem).wait()

        @pl.when(need_xb)
        def _():
            xb_copy().wait()

        br = lax.shift_right_logical(it, 2)
        qslot0 = (it * (NCI * NG)) & (QRING - 1)
        cont = (it & (ITB - 1)) != 0
        final = (it & (ITB - 1)) == ITB - 1
        qvals, pvals = {}, {}
        for kind, c, g, n in order:
            head = c * HC + n
            rows = pl.ds(g * M, M)
            cols = slice(n * DH, (n + 1) * DH)
            if kind == 'Q':
                blk = PC * NG + it * QG + g
                q_item(lax.shift_right_logical(blk, 6), lax.shift_right_logical(blk, 3),
                       pl.multiple_of((blk & (NG - 1)) * M, M), n, blk & (QRING - 1))
            elif kind == 'L':
                qvals[c, g, n] = q_s[qslot0 + c * NG + g, :, cols]
            elif kind == 'S':
                q = qvals.pop((c, g, n))
                ss = [lax.dot_general(q[j * SQ:(j + 1) * SQ], k_v[it, g * G + j, head],
                                      (((1,), (1,)), ((), ())), preferred_element_type=f32)
                      for j in range(G)]
                pvals[c, g, n] = [_softmax(s) for s in ss]
            elif kind == 'P':
                for j, p in enumerate(pvals.pop((c, g, n))):
                    b = g * G + j
                    o = jnp.dot(p, v_v[it, b, head], preferred_element_type=f32)
                    o_s[c, b * SQ:(b + 1) * SQ, cols] = o.astype(bf16)
            else:
                r = jnp.dot(o_s[c, rows, :], wo_v[it, c * CW:(c + 1) * CW, cols], preferred_element_type=f32)
                a = acc[rows, cols]
                if c == 0:
                    a = jnp.where(cont, a, 0.0)
                r = r + a
                acc[rows, cols] = r
                if c == NCI - 1:
                    rb = r.astype(bf16)
                    pieces = out_pieces(g, n)
                    if len(pieces) > 1:
                        for pc in pieces:
                            out_v[br, pl.ds(pc[0], pc[1]), cols] = rb[pc[0] - g * M:pc[0] - g * M + pc[1]]
                            pl.when(final)(lambda pc=pc: out_copy(br, *pc).start())
                    else:
                        out_v[br, rows, cols] = rb
                        for pc in pieces:
                            pl.when(final)(lambda pc=pc: out_copy(br, *pc).start())
        return carry

    lax.fori_loop(0, NIT, step, 0)
    for br in range(2):
        for g in range(NG):
            for n in range(HC):
                for pc in out_pieces(g, n):
                    out_copy(br, *pc).wait()


@jax.jit
def pallas_concat_heads__gqa_block_cached__gqa_block_cached__near_ridge_kernel(
    A_x: jax.Array,
    A_k_cache: jax.Array,
    A_v_cache: jax.Array,
    A_wq: jax.Array,
    A_wo: jax.Array,
    B_x: jax.Array,
    B_k_cache: jax.Array,
    B_v_cache: jax.Array,
    B_wq: jax.Array,
    B_wo: jax.Array,
):
    assert A_x.shape == (B, SQ, D) and A_k_cache.shape == (B, H, SQ, DH)
    hbm = pl.BlockSpec(memory_space=pl.ANY)
    out = pl.pallas_call(
        _body,
        in_specs=[hbm] * 10,
        out_specs=hbm,
        out_shape=jax.ShapeDtypeStruct((ROWS, 2 * D), bf16),
        scratch_shapes=[
            pltpu.VMEM((2, ROWS, D), bf16),
            pltpu.VMEM((NCH, D, CW), bf16),
            pltpu.VMEM((NIT, NCI * CW, D), bf16),
            pltpu.VMEM((NIT, B, NCI * HC, SQ, DH), bf16),
            pltpu.VMEM((NIT, B, NCI * HC, SQ, DH), bf16),
            pltpu.VMEM((QRING, M, CW), bf16),
            pltpu.VMEM((NCI, ROWS, CW), bf16),
            pltpu.VMEM((ROWS, D), f32),
            pltpu.VMEM((2, ROWS, D), bf16),
            pltpu.SemaphoreType.DMA((NIT + 1 + len(WAVES),)),
            pltpu.SemaphoreType.DMA((2,)),
        ],
        compiler_params=pltpu.CompilerParams(
            vmem_limit_bytes=110 * 1024 * 1024,
            disable_bounds_checks=True,
            disable_semaphore_checks=True,
        ),
    )(A_x.reshape(ROWS, D), A_k_cache, A_v_cache, A_wq, A_wo,
      B_x.reshape(ROWS, D), B_k_cache, B_v_cache, B_wq, B_wo)
    return out.reshape(B, SQ, 2 * D)
```

```python
import jax
import jax.numpy as jnp
from jax import lax
import jax.experimental.pallas as pl
import jax.experimental.pallas.tpu as pltpu

B = 32
H = 32
SQ = 48
DH = 128
D = 512
HC = 4
G = 4
NCI = 2
PC = 4
LK = 9
LP = 2
LO = 2
TAILR = 4

NG = B // G
NCB = H // HC
NCH = 2 * NCB
NIT = NCH // NCI
ITB = NCB // NCI
M = G * SQ
HM = M // 2
ROWS = B * SQ
CW = HC * DH
NU = NG * HC
QG = (NCH - PC) * NG // NIT
QRING = 64
NWQ = (NCH - PC) // NCI
XB_IT = 2
SCALE_LOG2E = (DH ** -0.5) * 1.4426950408889634
WAVES = ((2, 1), (3, 2), (4, 3), (5, 5), (8, 8), (2 * NG, PC * HC))

assert QG * NIT == (NCH - PC) * NG and ITB == 4 and NG == 8 and NCB * NG == 64
assert PC * NG + QG <= QRING
for _it in range(NIT):
    _last = PC * NG + QG * (_it + 1) - 1
    assert _last // NG < PC + NCI * (_it + 1)
    assert _it >= XB_IT or _last < NCB * NG

bf16 = jnp.bfloat16
f32 = jnp.float32


def _softmax(s):
    m = jnp.max(s, axis=-1, keepdims=True)
    e = jnp.exp2((s - m) * SCALE_LOG2E)
    l = jnp.sum(e, axis=-1, keepdims=True)
    r = pl.reciprocal(l, approx=True)
    r = r * (2.0 - l * r)
    return (e * r).astype(bf16)


def _loop_order():
    def units(kind):
        return [(kind, c, u // HC, u % HC) for c in range(NCI) for u in range(NU)]
    streams = ((LK, units('L')[LK:]), (0, units('S')), (-1, units('L')[:LK]),
               (0, [('Q', 0, j // HC, j % HC) for j in range(QG * HC)]),
               (LP + HC - 1 + LO, units('O')), (LP, units('P')))
    order = []
    for k in range(-1, max(off + len(items) for off, items in streams)):
        for off, items in streams:
            if 0 <= k - off < len(items):
                order.append(items[k - off])
    return order


def _body(ax, ak, av, awq, awo, bx, bk, bv, bwq, bwo, out_hbm,
          x_v, wq_v, wo_v, k_v, v_v, q_s, o_s, acc, out_v, sem_in, sem_out):
    srcs = ((ax, ak, av, awq, awo), (bx, bk, bv, bwq, bwo))
    copy = pltpu.make_async_copy

    def wave_copies(i):
        r0, h0 = WAVES[i - 1] if i else (0, 0)
        r1, h1 = WAVES[i]
        sem = sem_in.at[NIT + 1 + i]
        cps = []
        while h0 < h1:
            e = min(h1, (h0 // HC + 1) * HC)
            cps.append(copy(awq.at[:, pl.ds(h0 * DH, (e - h0) * DH)],
                            wq_v.at[h0 // HC, :, pl.ds((h0 % HC) * DH, (e - h0) * DH)], sem))
            h0 = e
        rows = pl.ds(r0 * HM, (r1 - r0) * HM)
        return cps + [copy(ax.at[rows], x_v.at[0, rows], sem)]

    def xb_copy():
        return copy(bx, x_v.at[1], sem_in.at[NIT])

    def out_copy(br, row0, nrows, col0, ncols):
        rows = pl.ds(row0, nrows)
        return copy(out_v.at[br, rows, pl.ds(col0, ncols)],
                    out_hbm.at[rows, pl.ds(pl.multiple_of(br * D + col0, DH), ncols)], sem_out.at[br])

    def out_pieces(g, n):
        if g < NG - 1:
            return [(g * M, M, 0, D)] if n == HC - 1 else []
        if n < HC - 1:
            return [(g * M, M, n * DH, DH)]
        return [(g * M + i * (M // TAILR), M // TAILR, n * DH, DH) for i in range(TAILR)]

    def q_item(br, c, row0, n, slot, r0=0, nr=M):
        cols = slice(n * DH, (n + 1) * DH)
        q = jnp.dot(x_v[br, pl.ds(row0, nr), :], wq_v[c, :, cols], preferred_element_type=f32)
        q_s[slot, n, r0:r0 + nr, :] = q.astype(bf16)

    for i in range(len(WAVES)):
        for cp in wave_copies(i):
            cp.start()
    for it in range(NIT):
        sem = sem_in.at[it]
        if it == XB_IT:
            xb_copy().start()
        if it < NWQ:
            for c in range(PC + it * NCI, PC + (it + 1) * NCI):
                copy(srcs[c // NCB][3].at[:, pl.ds((c % NCB) * CW, CW)], wq_v.at[c], sem).start()
        br, hc = it // ITB, (it % ITB) * NCI
        heads = pl.ds(hc * HC, NCI * HC)
        copy(srcs[br][1].at[:, heads], k_v.at[it], sem).start()
        copy(srcs[br][2].at[:, heads], v_v.at[it], sem).start()
        copy(srcs[br][4].at[pl.ds(hc * CW, NCI * CW), :], wo_v.at[it], sem).start()

    done = set()
    for i, (nr, nh) in enumerate(WAVES):
        for cp in wave_copies(i):
            cp.wait()
        for c, g, n in sorted((h // HC, g, h % HC) for h in range(nh) for g in range((nr + 1) // 2)):
            halves = [a for a in range(2) if 2 * g + a < nr and (c, g, n, a) not in done]
            if halves:
                q_item(0, c, g * M + halves[0] * HM, n, c * NG + g, halves[0] * HM, len(halves) * HM)
                done.update((c, g, n, a) for a in halves)

    order = _loop_order()

    def step(it, carry):
        sem = sem_in.at[it]
        need_wq, need_xb = it < NWQ, it == XB_IT
        for dst in (k_v.at[it], v_v.at[it], wo_v.at[it]):
            copy(dst, dst, sem).wait()

        @pl.when(need_wq)
        def _():
            dst = wq_v.at[pl.ds(jnp.minimum(PC + it * NCI, NCH - NCI), NCI)]
            copy(dst, dst, sem).wait()

        @pl.when(need_xb)
        def _():
            xb_copy().wait()

        br = lax.shift_right_logical(it, 2)
        qslot0 = (it * (NCI * NG)) & (QRING - 1)
        cont = (it & (ITB - 1)) != 0
        final = (it & (ITB - 1)) == ITB - 1
        qvals, pvals = {}, {}
        for kind, c, g, n in order:
            head = c * HC + n
            rows = pl.ds(g * M, M)
            cols = slice(n * DH, (n + 1) * DH)
            if kind == 'Q':
                blk = PC * NG + it * QG + g
                q_item(lax.shift_right_logical(blk, 6), lax.shift_right_logical(blk, 3),
                       pl.multiple_of((blk & (NG - 1)) * M, M), n, blk & (QRING - 1))
            elif kind == 'L':
                qvals[c, g, n] = q_s[qslot0 + c * NG + g, n]
            elif kind == 'S':
                q = qvals.pop((c, g, n))
                ss = [lax.dot_general(q[j * SQ:(j + 1) * SQ], k_v[it, g * G + j, head],
                                      (((1,), (1,)), ((), ())), preferred_element_type=f32)
                      for j in range(G)]
                pvals[c, g, n] = [_softmax(s) for s in ss]
            elif kind == 'P':
                for j, p in enumerate(pvals.pop((c, g, n))):
                    b = g * G + j
                    o = jnp.dot(p, v_v[it, b, head], preferred_element_type=f32)
                    o_s[c, n, b * SQ:(b + 1) * SQ, :] = o.astype(bf16)
            else:
                o = jnp.concatenate([o_s[c, h, rows, :] for h in range(HC)], axis=1)
                r = jnp.dot(o, wo_v[it, c * CW:(c + 1) * CW, cols], preferred_element_type=f32)
                a = acc[rows, cols]
                if c == 0:
                    a = jnp.where(cont, a, 0.0)
                r = r + a
                acc[rows, cols] = r
                if c == NCI - 1:
                    rb = r.astype(bf16)
                    pieces = out_pieces(g, n)
                    if len(pieces) > 1:
                        for pc in pieces:
                            out_v[br, pl.ds(pc[0], pc[1]), cols] = rb[pc[0] - g * M:pc[0] - g * M + pc[1]]
                            pl.when(final)(lambda pc=pc: out_copy(br, *pc).start())
                    else:
                        out_v[br, rows, cols] = rb
                        for pc in pieces:
                            pl.when(final)(lambda pc=pc: out_copy(br, *pc).start())
        return carry

    lax.fori_loop(0, NIT, step, 0)
    for br in range(2):
        for g in range(NG):
            for n in range(HC):
                for pc in out_pieces(g, n):
                    out_copy(br, *pc).wait()


@jax.jit
def pallas_concat_heads__gqa_block_cached__gqa_block_cached__near_ridge_kernel(
    A_x: jax.Array,
    A_k_cache: jax.Array,
    A_v_cache: jax.Array,
    A_wq: jax.Array,
    A_wo: jax.Array,
    B_x: jax.Array,
    B_k_cache: jax.Array,
    B_v_cache: jax.Array,
    B_wq: jax.Array,
    B_wo: jax.Array,
):
    assert A_x.shape == (B, SQ, D) and A_k_cache.shape == (B, H, SQ, DH)
    hbm = pl.BlockSpec(memory_space=pl.ANY)
    out = pl.pallas_call(
        _body,
        in_specs=[hbm] * 10,
        out_specs=hbm,
        out_shape=jax.ShapeDtypeStruct((ROWS, 2 * D), bf16),
        scratch_shapes=[
            pltpu.VMEM((2, ROWS, D), bf16),
            pltpu.VMEM((NCH, D, CW), bf16),
            pltpu.VMEM((NIT, NCI * CW, D), bf16),
            pltpu.VMEM((NIT, B, NCI * HC, SQ, DH), bf16),
            pltpu.VMEM((NIT, B, NCI * HC, SQ, DH), bf16),
            pltpu.VMEM((QRING, HC, M, DH), bf16),
            pltpu.VMEM((NCI, HC, ROWS, DH), bf16),
            pltpu.VMEM((ROWS, D), f32),
            pltpu.VMEM((2, ROWS, D), bf16),
            pltpu.SemaphoreType.DMA((NIT + 1 + len(WAVES),)),
            pltpu.SemaphoreType.DMA((2,)),
        ],
        compiler_params=pltpu.CompilerParams(
            vmem_limit_bytes=110 * 1024 * 1024,
            disable_bounds_checks=True,
            disable_semaphore_checks=True,
        ),
    )(A_x.reshape(ROWS, D), A_k_cache, A_v_cache, A_wq, A_wo,
      B_x.reshape(ROWS, D), B_k_cache, B_v_cache, B_wq, B_wo)
    return out.reshape(B, SQ, 2 * D)
```

```python
import jax
import jax.numpy as jnp
from jax import lax
import jax.experimental.pallas as pl
import jax.experimental.pallas.tpu as pltpu

B = 32
H = 32
SQ = 48
DH = 128
D = 512
HC = 4
G = 4
NCI = 2
PC = 4
LK = 9
LP = 2
LO = 2
TAILR = 4

NG = B // G
NCB = H // HC
NCH = 2 * NCB
NIT = NCH // NCI
ITB = NCB // NCI
M = G * SQ
HM = M // 2
ROWS = B * SQ
CW = HC * DH
NU = NG * HC
QG = (NCH - PC) * NG // NIT
QRING = 64
NWQ = (NCH - PC) // NCI
XB_IT = 2
SCALE_LOG2E = (DH ** -0.5) * 1.4426950408889634
WAVES = ((2, 1), (3, 2), (4, 3), (5, 5), (8, 8), (2 * NG, PC * HC))

assert QG * NIT == (NCH - PC) * NG and ITB == 4 and NG == 8 and NCB * NG == 64
assert PC * NG + QG <= QRING
for _it in range(NIT):
    _last = PC * NG + QG * (_it + 1) - 1
    assert _last // NG < PC + NCI * (_it + 1)
    assert _it >= XB_IT or _last < NCB * NG

bf16 = jnp.bfloat16
f32 = jnp.float32


def _softmax(s):
    m = jnp.max(s, axis=-1, keepdims=True)
    e = jnp.exp2((s - m) * SCALE_LOG2E)
    l = jnp.sum(e, axis=-1, keepdims=True)
    r = pl.reciprocal(l, approx=True)
    r = r * (2.0 - l * r)
    return (e * r).astype(bf16)


def _loop_order():
    def units(kind):
        return [(kind, c, u // HC, u % HC) for c in range(NCI) for u in range(NU)]
    streams = ((LK, units('L')[LK:]), (0, units('S')), (-1, units('L')[:LK]),
               (0, [('Q', 0, j // HC, j % HC) for j in range(QG * HC)]),
               (LP + HC - 1 + LO, units('O')), (LP, units('P')))
    order = []
    for k in range(-1, max(off + len(items) for off, items in streams)):
        for off, items in streams:
            if 0 <= k - off < len(items):
                order.append(items[k - off])
    pos = {item: i for i, item in enumerate(order)}
    for it in range(NIT):
        for _, c, g, n in units('L'):
            j = (it * NCI + c) * NG + g - (PC * NG + it * QG)
            assert j < 0 or pos['Q', 0, j, n] < pos['L', c, g, n]
    return order


def _body(ax, ak, av, awq, awo, bx, bk, bv, bwq, bwo, out_hbm,
          x_v, wq_v, wo_v, k_v, v_v, q_s, o_s, acc, out_v, sem_in, sem_out):
    srcs = ((ax, ak, av, awq, awo), (bx, bk, bv, bwq, bwo))
    copy = pltpu.make_async_copy

    def wave_copies(i):
        r0, h0 = WAVES[i - 1] if i else (0, 0)
        r1, h1 = WAVES[i]
        sem = sem_in.at[NIT + 1 + i]
        cps = []
        while h0 < h1:
            e = min(h1, (h0 // HC + 1) * HC)
            cps.append(copy(awq.at[:, pl.ds(h0 * DH, (e - h0) * DH)],
                            wq_v.at[h0 // HC, :, pl.ds((h0 % HC) * DH, (e - h0) * DH)], sem))
            h0 = e
        rows = pl.ds(r0 * HM, (r1 - r0) * HM)
        return cps + [copy(ax.at[rows], x_v.at[0, rows], sem)]

    def xb_copy():
        return copy(bx, x_v.at[1], sem_in.at[NIT])

    def out_copy(br, row0, nrows, col0, ncols):
        rows = pl.ds(row0, nrows)
        return copy(out_v.at[br, rows, pl.ds(col0, ncols)],
                    out_hbm.at[rows, pl.ds(pl.multiple_of(br * D + col0, DH), ncols)], sem_out.at[br])

    def out_pieces(g, n):
        if g < NG - 1:
            return [(g * M, M, 0, D)] if n == HC - 1 else []
        if n < HC - 1:
            return [(g * M, M, n * DH, DH)]
        return [(g * M + i * (M // TAILR), M // TAILR, n * DH, DH) for i in range(TAILR)]

    def q_item(br, c, row0, n, slot, r0=0, nr=M):
        cols = slice(n * DH, (n + 1) * DH)
        q = jnp.dot(x_v[br, pl.ds(row0, nr), :], wq_v[c, :, cols], preferred_element_type=f32)
        q_s[slot, n, r0:r0 + nr, :] = q.astype(bf16)

    for i in range(len(WAVES)):
        for cp in wave_copies(i):
            cp.start()
    for it in range(NIT):
        sem = sem_in.at[it]
        if it == XB_IT:
            xb_copy().start()
        if it < NWQ:
            for c in range(PC + it * NCI, PC + (it + 1) * NCI):
                copy(srcs[c // NCB][3].at[:, pl.ds((c % NCB) * CW, CW)], wq_v.at[c], sem).start()
        br, hc = it // ITB, (it % ITB) * NCI
        heads = pl.ds(hc * HC, NCI * HC)
        copy(srcs[br][1].at[:, heads], k_v.at[it], sem).start()
        copy(srcs[br][2].at[:, heads], v_v.at[it], sem).start()
        copy(srcs[br][4].at[pl.ds(hc * CW, NCI * CW), :], wo_v.at[it], sem).start()

    done = set()
    for i, (nr, nh) in enumerate(WAVES):
        for cp in wave_copies(i):
            cp.wait()
        for c, g, n in sorted((h // HC, g, h % HC) for h in range(nh) for g in range((nr + 1) // 2)):
            halves = [a for a in range(2) if 2 * g + a < nr and (c, g, n, a) not in done]
            if halves:
                q_item(0, c, g * M + halves[0] * HM, n, c * NG + g, halves[0] * HM, len(halves) * HM)
                done.update((c, g, n, a) for a in halves)

    order = _loop_order()

    def step(it, carry):
        sem = sem_in.at[it]
        need_wq, need_xb = it < NWQ, it == XB_IT
        for dst in (k_v.at[it], v_v.at[it], wo_v.at[it]):
            copy(dst, dst, sem).wait()

        @pl.when(need_wq)
        def _():
            dst = wq_v.at[pl.ds(jnp.minimum(PC + it * NCI, NCH - NCI), NCI)]
            copy(dst, dst, sem).wait()

        @pl.when(need_xb)
        def _():
            xb_copy().wait()

        br = lax.shift_right_logical(it, 2)
        qslot0 = (it * (NCI * NG)) & (QRING - 1)
        cont = (it & (ITB - 1)) != 0
        final = (it & (ITB - 1)) == ITB - 1
        qvals, pvals = {}, {}
        for kind, c, g, n in order:
            head = c * HC + n
            rows = pl.ds(g * M, M)
            cols = slice(n * DH, (n + 1) * DH)
            if kind == 'Q':
                blk = PC * NG + it * QG + g
                q_item(lax.shift_right_logical(blk, 6), lax.shift_right_logical(blk, 3),
                       pl.multiple_of((blk & (NG - 1)) * M, M), n, blk & (QRING - 1))
            elif kind == 'L':
                qvals[c, g, n] = q_s[qslot0 + c * NG + g, n]
            elif kind == 'S':
                q = qvals.pop((c, g, n))
                ss = [lax.dot_general(q[j * SQ:(j + 1) * SQ], k_v[it, g * G + j, head],
                                      (((1,), (1,)), ((), ())), preferred_element_type=f32)
                      for j in range(G)]
                pvals[c, g, n] = [_softmax(s) for s in ss]
            elif kind == 'P':
                for j, p in enumerate(pvals.pop((c, g, n))):
                    b = g * G + j
                    o = jnp.dot(p, v_v[it, b, head], preferred_element_type=f32)
                    o_s[c, n, b * SQ:(b + 1) * SQ, :] = o.astype(bf16)
            else:
                o = jnp.concatenate([o_s[c, h, rows, :] for h in range(HC)], axis=1)
                r = jnp.dot(o, wo_v[it, c * CW:(c + 1) * CW, cols], preferred_element_type=f32)
                a = acc[rows, cols]
                if c == 0:
                    a = jnp.where(cont, a, 0.0)
                r = r + a
                acc[rows, cols] = r
                if c == NCI - 1:
                    rb = r.astype(bf16)
                    pieces = out_pieces(g, n)
                    if len(pieces) > 1:
                        for pc in pieces:
                            out_v[br, pl.ds(pc[0], pc[1]), cols] = rb[pc[0] - g * M:pc[0] - g * M + pc[1]]
                            pl.when(final)(lambda pc=pc: out_copy(br, *pc).start())
                    else:
                        out_v[br, rows, cols] = rb
                        for pc in pieces:
                            pl.when(final)(lambda pc=pc: out_copy(br, *pc).start())
        return carry

    lax.fori_loop(0, NIT, step, 0)
    for br in range(2):
        for g in range(NG):
            for n in range(HC):
                for pc in out_pieces(g, n):
                    out_copy(br, *pc).wait()


@jax.jit
def pallas_concat_heads__gqa_block_cached__gqa_block_cached__near_ridge_kernel(
    A_x: jax.Array,
    A_k_cache: jax.Array,
    A_v_cache: jax.Array,
    A_wq: jax.Array,
    A_wo: jax.Array,
    B_x: jax.Array,
    B_k_cache: jax.Array,
    B_v_cache: jax.Array,
    B_wq: jax.Array,
    B_wo: jax.Array,
):
    assert A_x.shape == (B, SQ, D) and A_k_cache.shape == (B, H, SQ, DH)
    hbm = pl.BlockSpec(memory_space=pl.ANY)
    out = pl.pallas_call(
        _body,
        in_specs=[hbm] * 10,
        out_specs=hbm,
        out_shape=jax.ShapeDtypeStruct((ROWS, 2 * D), bf16),
        scratch_shapes=[
            pltpu.VMEM((2, ROWS, D), bf16),
            pltpu.VMEM((NCH, D, CW), bf16),
            pltpu.VMEM((NIT, NCI * CW, D), bf16),
            pltpu.VMEM((NIT, B, NCI * HC, SQ, DH), bf16),
            pltpu.VMEM((NIT, B, NCI * HC, SQ, DH), bf16),
            pltpu.VMEM((QRING, HC, M, DH), bf16),
            pltpu.VMEM((NCI, HC, ROWS, DH), bf16),
            pltpu.VMEM((ROWS, D), f32),
            pltpu.VMEM((2, ROWS, D), bf16),
            pltpu.SemaphoreType.DMA((NIT + 1 + len(WAVES),)),
            pltpu.SemaphoreType.DMA((2,)),
        ],
        compiler_params=pltpu.CompilerParams(
            vmem_limit_bytes=110 * 1024 * 1024,
            disable_bounds_checks=True,
            disable_semaphore_checks=True,
        ),
    )(A_x.reshape(ROWS, D), A_k_cache, A_v_cache, A_wq, A_wo,
      B_x.reshape(ROWS, D), B_k_cache, B_v_cache, B_wq, B_wo)
    return out.reshape(B, SQ, 2 * D)
```
